```python
import jax
import jax.numpy as jnp

def _softmax(x, axis=-1):
    return jax.nn.softmax(x, axis=axis)

def _gelu(x):
    return jax.nn.gelu(x, approximate=True)

def _silu(x):
    return jax.nn.silu(x)

def _sigmoid(x):
    return jax.nn.sigmoid(x)

def _layernorm(x, axis=-1, eps=1e-05):
    m = jnp.mean(x, axis=axis, keepdims=True)
    v = jnp.var(x, axis=axis, keepdims=True)
    return (x - m) / jnp.sqrt(v + eps)

def _scatter_add(tgt, idx, src, axis=0):
    return tgt.at[idx].add(src)

def _segment_sum(src, seg, n):
    return jax.ops.segment_sum(src, seg, n)

class _Rng:

    def __init__(self, key):
        self._k = key

    def _next(self):
        self._k, sub = jax.random.split(self._k)
        return sub

    def normal(self, shape):
        return jax.random.normal(self._next(), shape, dtype=jnp.bfloat16)

    def randint(self, lo, hi, shape):
        return jax.random.randint(self._next(), shape, lo, hi, dtype=jnp.int32)

    def uniform(self, shape, lo=0.0, hi=1.0):
        return jax.random.uniform(self._next(), shape, jnp.bfloat16, lo, hi)

    def permutation(self, n):
        return jax.random.permutation(self._next(), n)
kernel_name = 'adaLN_cond__sliding_block_cached__glu_gated_swiglu__decode'

def setup_inputs():
    _rng = _Rng(jax.random.key(int.from_bytes(__import__("os").urandom(4), "little")))
    _w = lambda a: (lambda t: t.astype(jnp.bfloat16) if jnp.issubdtype(t.dtype, jnp.floating) else t)(jnp.asarray(a))

    def _A_setup():
        B, Sq, D = (2, 1, 512)
        Hq, Hkv, Sk, Dh = (32, 32, 16384, 128)
        assert Hq % Hkv == 0, (Hq, Hkv)
        return {'x': _w((lambda *s: _rng.normal(s) * 0.05)(B, Sq, D)), 'k_cache': _w((lambda *s: _rng.normal(s) * 0.05)(B, Hkv, Sk, Dh)), 'v_cache': _w((lambda *s: _rng.normal(s) * 0.05)(B, Hkv, Sk, Dh)), 'wq': _w((lambda *s: _rng.normal(s) * 0.05)(D, Hq * Dh) * D ** (-0.5)), 'wo': _w((lambda *s: _rng.normal(s) * 0.05)(Hq * Dh, D) * (Hq * Dh) ** (-0.5))}
    _A_in = _A_setup()

    def _B_setup():
        B, S, D, F = (2, 1, 512, 1376)
        return {'x': _w((lambda *s: _rng.normal(s) * 0.05)(B, S, D)), 'w1': _w((lambda *s: _rng.normal(s) * 0.05)(D, F) * (2.0 / D) ** 0.5), 'w3': _w((lambda *s: _rng.normal(s) * 0.05)(D, F) * (2.0 / D) ** 0.5), 'w2': _w((lambda *s: _rng.normal(s) * 0.05)(F, D) * (2.0 / F) ** 0.5)}
    _B_in = _B_setup()
    return {'A_x': _A_in['x'], 'A_k_cache': _A_in['k_cache'], 'A_v_cache': _A_in['v_cache'], 'A_wq': _A_in['wq'], 'A_wo': _A_in['wo'], 'B_x': _B_in['x'], 'B_w1': _B_in['w1'], 'B_w3': _B_in['w3'], 'B_w2': _B_in['w2'], 'c': _w((lambda *s: _rng.normal(s) * 0.05)(2, 512)), 'w_mod': _w((lambda *s: _rng.normal(s) * 0.05)(512, 6 * 512) * 512 ** (-0.5))}

def reference(A_x, A_k_cache, A_v_cache, A_wq, A_wo, B_x, B_w1, B_w3, B_w2, c, w_mod):

    def _A_ref(x, k_cache, v_cache, wq, wo):
        B, Sq, D = x.shape
        Hq, Dh = (32, 128)
        Hkv, Sk = (k_cache.shape[1], k_cache.shape[2])
        W = min(4096, max(256, Sk // 4))
        rep = Hq // Hkv
        q = (lambda x, *d: x.transpose(*d))((x @ wq).reshape(B, Sq, Hq, Dh), 0, 2, 1, 3)
        k = jnp.repeat(k_cache[:, :, Sk - W:, :], rep, axis=1)
        v = jnp.repeat(v_cache[:, :, Sk - W:, :], rep, axis=1)
        scores = jnp.einsum('bhqd,bhkd->bhqk', q, k) * Dh ** (-0.5)
        p = _softmax(scores, axis=-1)
        o = jnp.einsum('bhqk,bhkd->bhqd', p, v)
        return (lambda x, *d: x.transpose(*d))(o, 0, 2, 1, 3).reshape(B, Sq, Hq * Dh) @ wo

    def _B_ref(x, w1, w3, w2):
        gate = jnp.einsum('bsd,df->bsf', x, w1)
        up = jnp.einsum('bsd,df->bsf', x, w3)
        h = _silu(gate) * up
        out = jnp.einsum('bsf,fd->bsd', h, w2)
        return out
    x = A_x
    mod = (_silu(c) @ w_mod).reshape(c.shape[0], 6, 1, -1)
    sa, ca, ga, sb, cb, gb = (mod[:, 0].copy(), mod[:, 1].copy(), mod[:, 2].copy(), mod[:, 3].copy(), mod[:, 4].copy(), mod[:, 5].copy())
    h = _layernorm(x, axis=-1) * (1 + ca) + sa
    x = x + ga * _A_ref(h, A_k_cache, A_v_cache, A_wq, A_wo)
    h = _layernorm(x, axis=-1) * (1 + cb) + sb
    x = x + gb * _B_ref(h, B_w1, B_w3, B_w2)
    return x
```

```python
import jax
import jax.numpy as jnp
from jax import lax
import jax.experimental.pallas as pl
import jax.experimental.pallas.tpu as pltpu

_BF = jnp.bfloat16
_F32 = jnp.float32
_NT = (((1,), (1,)), ((), ()))


def _layernorm(x, eps=1e-5):
    m = jnp.mean(x, axis=-1, keepdims=True)
    d = x - m
    v = jnp.mean(d * d, axis=-1, keepdims=True)
    return d / jnp.sqrt(v + eps)


def _silu(x):
    return x * jax.nn.sigmoid(x)


def _pad8(x):
    return jnp.concatenate([x, jnp.zeros((8 - x.shape[0], x.shape[1]), x.dtype)], axis=0)


@jax.jit
def pallas_adaLN_cond__sliding_block_cached__glu_gated_swiglu__decode_kernel(
    A_x, A_k_cache, A_v_cache, A_wq, A_wo, B_x, B_w1, B_w3, B_w2, c, w_mod,
):
    B, Sq, D = A_x.shape
    _, H, Sk, Dh = A_k_cache.shape
    F = B_w2.shape[0]
    W = min(4096, max(256, Sk // 4))
    S0 = Sk - W
    G = B * H
    NB = 3
    scale = Dh ** (-0.5)

    def kernel(x_hbm, k_hbm, v_hbm, wq_hbm, wo_hbm, w1_hbm, w3_hbm, w2_hbm, c_hbm, wm_hbm,
               o_ref,
               x_v, c_v, wm_v, wq_v, wo_v, w1_v, w3_v, w2_v, k_v, v_v, q_s, o_s,
               sem, ksem, vsem):
        def kcopy(g):
            s = g % NB
            return pltpu.make_async_copy(k_hbm.at[g // H, g % H, pl.ds(S0, W)], k_v.at[s], ksem.at[s])

        def vcopy(g):
            s = g % NB
            return pltpu.make_async_copy(v_hbm.at[g // H, g % H, pl.ds(S0, W)], v_v.at[s], vsem.at[s])

        cp_c = pltpu.make_async_copy(c_hbm, c_v, sem.at[0])
        cp_x = pltpu.make_async_copy(x_hbm, x_v, sem.at[1])
        cp_wm = pltpu.make_async_copy(wm_hbm, wm_v, sem.at[2])
        cp_wq = pltpu.make_async_copy(wq_hbm, wq_v, sem.at[3])
        cp_wo = pltpu.make_async_copy(wo_hbm, wo_v, sem.at[4])
        cp_w1 = pltpu.make_async_copy(w1_hbm, w1_v, sem.at[5])
        cp_w3 = pltpu.make_async_copy(w3_hbm, w3_v, sem.at[6])
        cp_w2 = pltpu.make_async_copy(w2_hbm, w2_v, sem.at[7])

        cp_c.start()
        cp_x.start()
        cp_wm.start()
        cp_wq.start()
        for g in range(NB):
            kcopy(g).start()
            vcopy(g).start()

        cp_c.wait()
        cp_x.wait()
        sc = _pad8(_silu(c_v[...].astype(_F32))).astype(_BF)
        x = _pad8(x_v[...].astype(_F32))
        cp_wm.wait()
        mod = jnp.dot(sc, wm_v[...], preferred_element_type=_F32)
        sa, ca, ga, sb, cb, gb = (mod[:, i * D:(i + 1) * D] for i in range(6))
        h = _layernorm(x) * (1.0 + ca) + sa
        cp_wq.wait()
        q = jnp.dot(h.astype(_BF), wq_v[...], preferred_element_type=_F32)
        for b in range(B):
            for hh in range(H):
                q_s[b * H + hh] = jnp.broadcast_to(q[b:b + 1, hh * Dh:(hh + 1) * Dh], (8, Dh))

        def head(g, _):
            s = g % NB
            kcopy(g).wait()
            qg = q_s[g].astype(_BF)
            sc_ = lax.dot_general(qg, k_v[s], _NT, preferred_element_type=_F32) * scale

            @pl.when(g + NB < G)
            def _():
                kcopy(g + NB).start()

            @pl.when(g == G - NB)
            def _():
                cp_wo.start()
                cp_w1.start()
                cp_w3.start()
                cp_w2.start()

            m = jnp.max(sc_, axis=-1, keepdims=True)
            p = jnp.exp(sc_ - m)
            l = jnp.sum(p, axis=-1, keepdims=True)
            vcopy(g).wait()
            o = jnp.dot(p.astype(_BF), v_v[s], preferred_element_type=_F32) / l
            o_s[g] = o

            @pl.when(g + NB < G)
            def _():
                vcopy(g + NB).start()

        lax.fori_loop(0, G, head, None)

        row = lax.broadcasted_iota(jnp.int32, (8, Dh), 0)
        cols = []
        for hh in range(H):
            t = jnp.zeros((8, Dh), _F32)
            for b in range(B):
                t = jnp.where(row == b, o_s[b * H + hh], t)
            cols.append(t)
        o_all = jnp.concatenate(cols, axis=1).astype(_BF)
        cp_wo.wait()
        attn = jnp.dot(o_all, wo_v[...], preferred_element_type=_F32)
        x = x + ga * attn
        h2 = (_layernorm(x) * (1.0 + cb) + sb).astype(_BF)
        cp_w1.wait()
        gate = lax.dot_general(h2, w1_v[...], _NT, preferred_element_type=_F32)
        cp_w3.wait()
        up = lax.dot_general(h2, w3_v[...], _NT, preferred_element_type=_F32)
        hm = (_silu(gate) * up).astype(_BF)
        cp_w2.wait()
        ffn = jnp.dot(hm, w2_v[...], preferred_element_type=_F32)
        x = x + gb * ffn
        o_ref[...] = x[:B].astype(o_ref.dtype)

    hbm = pl.BlockSpec(memory_space=pltpu.HBM)
    out = pl.pallas_call(
        kernel,
        out_shape=jax.ShapeDtypeStruct((B, D), A_x.dtype),
        in_specs=[hbm] * 10,
        out_specs=pl.BlockSpec(memory_space=pltpu.VMEM),
        scratch_shapes=[
            pltpu.VMEM((B, D), _BF), pltpu.VMEM((B, D), _BF),
            pltpu.VMEM(w_mod.shape, _BF), pltpu.VMEM(A_wq.shape, _BF), pltpu.VMEM(A_wo.shape, _BF),
            pltpu.VMEM((F, D), _BF), pltpu.VMEM((F, D), _BF), pltpu.VMEM((F, D), _BF),
            pltpu.VMEM((NB, W, Dh), _BF), pltpu.VMEM((NB, W, Dh), _BF),
            pltpu.VMEM((G, 8, Dh), _F32), pltpu.VMEM((G, 8, Dh), _F32),
            pltpu.SemaphoreType.DMA((8,)), pltpu.SemaphoreType.DMA((NB,)), pltpu.SemaphoreType.DMA((NB,)),
        ],
        compiler_params=pltpu.CompilerParams(vmem_limit_bytes=64 * 1024 * 1024),
    )(A_x.reshape(B, D), A_k_cache, A_v_cache, A_wq, A_wo, B_w1.T, B_w3.T, B_w2, c, w_mod)
    return out.reshape(B, Sq, D)
```

```python
import functools

import jax
import jax.numpy as jnp
from jax import lax
import jax.experimental.pallas as pl
import jax.experimental.pallas.tpu as pltpu

_BF = jnp.bfloat16
_F32 = jnp.float32
_NT = (((1,), (1,)), ((), ()))

LAG = 6
RING = 8


def _layernorm(x, eps=1e-5):
    m = jnp.mean(x, axis=-1, keepdims=True)
    d = x - m
    v = jnp.mean(d * d, axis=-1, keepdims=True)
    return d / jnp.sqrt(v + eps)


def _silu(x):
    return x * jax.nn.sigmoid(x)


def _block(i, n):
    return pl.ds(i * n if isinstance(i, int) else pl.multiple_of(i * n, n), n)


def _wait_all(buf, sem):
    pltpu.make_async_copy(buf, buf, sem).wait()


@jax.jit
def pallas_adaLN_cond__sliding_block_cached__glu_gated_swiglu__decode_kernel(
    A_x: jax.Array,
    A_k_cache: jax.Array,
    A_v_cache: jax.Array,
    A_wq: jax.Array,
    A_wo: jax.Array,
    B_x: jax.Array,
    B_w1: jax.Array,
    B_w3: jax.Array,
    B_w2: jax.Array,
    c: jax.Array,
    w_mod: jax.Array,
):
    del B_x
    B, Sq, D = A_x.shape
    _, H, Sk, Dh = A_k_cache.shape
    F = B_w2.shape[0]
    W = min(4096, max(256, Sk // 4))
    S0 = Sk - W
    scale = Dh ** (-0.5)
    R = 128
    PR = 64
    WR = 16
    NC = W // R
    NG = H // 2
    CB = 1024
    NMOD, NQ = 6 * D // CB, H * Dh // CB
    FC = 256
    NF, FR = F // FC, F % FC
    assert (B, Sq, D, H, Dh, NC, NF, FR) == (2, 1, 512, 32, 128, 32, 5, 96)

    T_Q = 4 * NMOD
    T_K0 = T_Q + 4 * NQ
    T_KV = T_K0 + NC
    T_VL = T_KV + (NG - 1) * NC
    T_F1 = T_VL + NC // 2
    T_F2 = T_F1 + 1 + 2 * NF
    T_END = T_F2 + 1 + NF

    def kernel(x_hbm, k_hbm, v_hbm, wq_hbm, wo_hbm, w1_hbm, w3_hbm, w2_hbm, c_hbm, wm_hbm,
               o_ref,
               cx_v, wc_v, wo_v, w13_v, w2_v, kv_v, q_s, s_s, h_s, sems, wo_sem):
        row = lax.broadcasted_iota(jnp.int32, (8, Dh), 0)

        def sem(t):
            return sems.at[t & (RING - 1)]

        def wc_sem(n):
            return sem(T_K0 + 1 + n)

        def w13_sem(n):
            return sem(T_F1 + n)

        def w2_sem(n):
            return sem(T_F1 + NF + 1 + n)

        def kv_piece(ref, g, s, i, e, t, u):
            head = (s & 1) * H + 2 * g + (s >> 1)
            src = ref.at[_block(head * (Sk // PR) + S0 // PR + i * (R // PR) + e, PR)]
            return src, kv_v.at[t & (RING - 1), u, _block(e, PR)], sem(t)

        def pairs(first, second):
            return [f(s, e) for e in range(2) for s in range(4) for f in (first, second)]

        def st_cols(src, base):
            def f(i, t):
                n = i >> 2
                rows = [_block(((i & 3) + 4 * u) * 2 + e, 8) for e in range(2) for u in range(8)]
                return [(src.at[r, _block(n, CB)], wc_v.at[base + n, r], wc_sem(base + n)) for r in rows]
            return f

        def st_k0(i, t):
            def wo_piece(s, e):
                r = _block((s * NC + i) * 2 + e, WR)
                return wo_hbm.at[r], wo_v.at[r], wo_sem
            return pairs(lambda s, e: kv_piece(k_hbm, 0, s, i, e, t, s), wo_piece)

        def st_kv(i, t):
            g, i = i >> 5, i & (NC - 1)
            return pairs(lambda s, e: kv_piece(k_hbm, g + 1, s, i, e, t, s),
                         lambda s, e: kv_piece(v_hbm, g, s, i, e, t, 4 + s))

        def st_vl(i, t):
            return pairs(lambda s, e: kv_piece(v_hbm, NG - 1, s, i, e, t, s),
                         lambda s, e: kv_piece(v_hbm, NG - 1, s, i + NC // 2, e, t, 4 + s))

        def w13_piece(j, p, n):
            r = _block(p, WR)
            return (w1_hbm, w3_hbm)[j].at[r], w13_v.at[j, r], w13_sem(n)

        def w2_piece(p, n):
            r = _block(p, WR)
            return w2_hbm.at[r], w2_v.at[r], w2_sem(n)

        ragged = range(NF * FC // WR, F // WR)

        def st_w13(i, t):
            p0 = (i >> 1) * (FC // WR) + (i & 1) * 2
            return pairs(lambda s, e: w13_piece(0, p0 + 4 * s + e, 1 + (i >> 1)),
                         lambda s, e: w13_piece(1, p0 + 4 * s + e, 1 + (i >> 1)))

        def st_w2(i, t):
            return [w2_piece(i * (FC // WR) + 2 * s + e, 1 + i) for e in range(2) for s in range(8)]

        stages = [
            (0, st_cols(wm_hbm, 0)),
            (T_Q, st_cols(wq_hbm, NMOD)),
            (T_K0, st_k0),
            (T_KV, st_kv),
            (T_VL, st_vl),
            (T_F1, lambda i, t: [w13_piece(j, p, 0) for p in ragged for j in range(2)]),
            (T_F1 + 1, st_w13),
            (T_F2, lambda i, t: [w2_piece(p, 0) for p in ragged]),
            (T_F2 + 1, st_w2),
        ]

        def step(stage, t, slot_fn=None):
            pieces = stage[1](t + LAG - stage[0], t + LAG)
            for u in range(8):
                for j in range(2 * u, min(2 * u + 2, len(pieces))):
                    pltpu.make_async_copy(*pieces[j]).start(priority=j & 1)
                if slot_fn is not None:
                    slot_fn(u)

        def run(t0, t1, body=None, carry=None, off=0):
            cuts = sorted({t0, t1} | {s - LAG for s, _ in stages if t0 < s - LAG < t1})
            for a, b in zip(cuts[:-1], cuts[1:]):
                stage = [st for st in stages if st[0] <= a + LAG][-1]

                def it(t, cr, stage=stage):
                    if body is None:
                        return step(stage, t)
                    return body(t, cr, functools.partial(step, stage, t))

                if b - a == 1:
                    carry = it(a + off, carry)
                else:
                    carry = lax.fori_loop(a + off, b + off, it, carry)
            return carry

        pltpu.make_async_copy(c_hbm, cx_v.at[0], wc_sem(-1)).start()
        pltpu.make_async_copy(x_hbm, cx_v.at[1], wc_sem(-1)).start()
        run(-LAG, 0)
        _wait_all(cx_v, wc_sem(-1))
        even = (lax.broadcasted_iota(jnp.int32, (8, D), 0) & 1) == 0

        def rep(v):
            v = v.astype(_F32)
            return jnp.where(even, v[0:1], v[1:2])

        sc = _silu(rep(cx_v[0])).astype(_BF)
        x = rep(cx_v[1])
        xn = _layernorm(x)
        mods = []
        for n in range(NMOD):
            run(4 * n, 4 * n + 4)
            _wait_all(wc_v.at[n], wc_sem(n))
            r = jnp.dot(sc, wc_v[n], preferred_element_type=_F32)
            mods += [r[:, :D], r[:, D:]]
        sa, ca, ga, sb, cb, gb = mods
        h = (xn * (1.0 + ca) + sa).astype(_BF)
        gpb = CB // (2 * Dh)
        for n in range(NQ):
            run(T_Q + 4 * n, T_Q + 4 * n + 4)
            _wait_all(wc_v.at[NMOD + n], wc_sem(NMOD + n))
            r = jnp.dot(h, wc_v[NMOD + n], preferred_element_type=_F32)
            for j in range(gpb):
                q_s[n * gpb + j] = jnp.where(row < 2, r[:, 2 * j * Dh:(2 * j + 1) * Dh],
                                             r[:, (2 * j + 1) * Dh:(2 * j + 2) * Dh])

        def qk(q, slot, u):
            return lax.dot_general(q, kv_v[slot, u], _NT, preferred_element_type=_F32)

        def pv(p, slot, u):
            return jnp.dot(p, kv_v[slot, u], preferred_element_type=_F32)

        def merge(rs):
            return jnp.where(row < 2, jnp.where(row == 0, rs[0], rs[1]), jnp.where(row == 2, rs[2], rs[3]))

        def body_k(q, tbase):
            def body(t, mx, issue):
                slot = t & (RING - 1)
                _wait_all(kv_v.at[slot, pl.ds(0, 4)], sem(t))
                rs = []
                issue(lambda u: None if u & 1 else rs.append(qk(q, slot, u >> 1)))
                s = merge(rs) * scale
                s_s[t - tbase] = s
                return jnp.maximum(mx, s)
            return body

        def body_kv(q, m, tbase):
            def body(t, cr, issue):
                mx, l, acc = cr
                slot = t & (RING - 1)
                _wait_all(kv_v.at[slot], sem(t))
                p = jnp.exp(s_s[t - tbase] - m)
                pb = p.astype(_BF)
                rs, acc = [], list(acc)

                def slot_fn(u):
                    if u & 1:
                        acc[u >> 1] += pv(pb, slot, 4 + (u >> 1))
                    else:
                        rs.append(qk(q, slot, u >> 1))

                issue(slot_fn)
                s = merge(rs) * scale
                s_s[t - tbase] = s
                return jnp.maximum(mx, s), l + p, tuple(acc)
            return body

        def body_v(m, tbase):
            def body(t, cr, issue):
                l, acc = cr
                slot = t & (RING - 1)
                _wait_all(kv_v.at[slot], sem(t))
                p0 = jnp.exp(s_s[t - tbase] - m)
                p1 = jnp.exp(s_s[t - tbase + NC // 2] - m)
                pb = (p0.astype(_BF), p1.astype(_BF))
                acc = list(acc)

                def slot_fn(u):
                    acc[u >> 1] += pv(pb[u & 1], slot, 4 * (u & 1) + (u >> 1))

                issue(slot_fn)
                return l + p0 + p1, tuple(acc)
            return body

        neg = jnp.full((8, Dh), -jnp.inf, _F32)
        zero = jnp.zeros((8, Dh), _F32)

        def rowmax(mx):
            return jnp.broadcast_to(jnp.max(mx, axis=-1, keepdims=True), (8, Dh))

        def project(g, l, acc):
            o = merge(acc) / jnp.sum(l, axis=-1, keepdims=True)
            o = jnp.concatenate([jnp.where(row < 2, o, 0.0),
                                 jnp.where((row >= 2) & (row < 4), o, 0.0)], axis=1)
            return jnp.dot(o.astype(_BF), wo_v[_block(g, 2 * Dh)], preferred_element_type=_F32)

        def phase(g, cr):
            m, attn = cr
            static = isinstance(g, int)
            t0, off = (T_KV + g * NC, 0) if static else (T_KV, g * NC)
            mx, l, acc = run(t0, t0 + NC, body_kv(q_s[g + 1].astype(_BF), m, t0 + off),
                             (neg, zero, (zero,) * 4), off)
            if not static:
                pl.when(g == 0)(lambda: _wait_all(wo_v, wo_sem))
            return rowmax(mx), attn + project(g, l, acc)

        mx = run(T_K0, T_KV, body_k(q_s[0].astype(_BF), T_K0), neg)
        m, attn = lax.fori_loop(0, NG - 2, phase, (rowmax(mx), jnp.zeros((8, D), _F32)))
        m, attn = phase(NG - 2, (m, attn))
        l, acc = run(T_VL, T_F1, body_v(m, T_VL), (zero, (zero,) * 4))
        attn = attn + project(NG - 1, l, acc)
        attn = attn + pltpu.roll(attn, 6, 0)
        x1 = x + ga * attn
        h2 = (_layernorm(x1) * (1.0 + cb) + sb).astype(_BF)

        def glu(rows, n):
            _wait_all(w13_v.at[:, rows], w13_sem(n))
            gate = lax.dot_general(h2, w13_v[0, rows], _NT, preferred_element_type=_F32)
            up = lax.dot_general(h2, w13_v[1, rows], _NT, preferred_element_type=_F32)
            return _silu(gate) * up

        def down(hm, rows, n):
            _wait_all(w2_v.at[rows], w2_sem(n))
            return jnp.dot(hm.astype(_BF), w2_v[rows], preferred_element_type=_F32)

        run(T_F1, T_F2 + 1 - LAG)
        h_rest = glu(pl.ds(NF * FC, FR), 0)

        def glu_chunk(i, _):
            step(stages[-1], T_F2 + 1 - LAG + i)
            h_s[i] = glu(_block(i, FC), 1 + i)

        lax.fori_loop(0, T_END - T_F2 - 1, glu_chunk, None)
        ffn = lax.fori_loop(0, NF, lambda i, a: a + down(h_s[i], _block(i, FC), 1 + i),
                            down(h_rest, pl.ds(NF * FC, FR), 0))
        o_ref[...] = (x1 + gb * ffn)[:B].astype(o_ref.dtype)

    hbm = pl.BlockSpec(memory_space=pltpu.HBM)
    out = pl.pallas_call(
        kernel,
        out_shape=jax.ShapeDtypeStruct((B, D), A_x.dtype),
        in_specs=[hbm] * 10,
        out_specs=pl.BlockSpec(memory_space=pltpu.VMEM),
        scratch_shapes=[
            pltpu.VMEM((2, B, D), _BF),
            pltpu.VMEM((NMOD + NQ, D, CB), _BF),
            pltpu.VMEM((H * Dh, D), _BF),
            pltpu.VMEM((2, F, D), _BF),
            pltpu.VMEM((F, D), _BF),
            pltpu.VMEM((RING, 8, R, Dh), _BF),
            pltpu.VMEM((NG, 8, Dh), _F32),
            pltpu.VMEM((NC, 8, Dh), _F32),
            pltpu.VMEM((NF, 8, FC), _F32),
            pltpu.SemaphoreType.DMA((RING,)),
            pltpu.SemaphoreType.DMA(()),
        ],
        compiler_params=pltpu.CompilerParams(vmem_limit_bytes=48 * 1024 * 1024),
    )(A_x.reshape(B, D), A_k_cache.reshape(B * H * Sk, Dh), A_v_cache.reshape(B * H * Sk, Dh),
      A_wq, A_wo, B_w1.T, B_w3.T, B_w2, c, w_mod)
    return out.reshape(B, Sq, D)
```
